```python
import os as _os
_os.environ.setdefault("JAX_PLATFORMS", "cpu")
import jax
import jax.numpy as jnp

def _softmax(x, axis=-1):
    return jax.nn.softmax(x, axis=axis)
def _gelu(x):
    return jax.nn.gelu(x, approximate=True)
def _silu(x):
    return jax.nn.silu(x)
def _sigmoid(x):
    return jax.nn.sigmoid(x)
def _layernorm(x, axis=-1, eps=1e-5):
    m = jnp.mean(x, axis=axis, keepdims=True)
    v = jnp.var(x, axis=axis, keepdims=True)
    return (x - m) / jnp.sqrt(v + eps)
def _scatter_add(tgt, idx, src, axis=0):
    return tgt.at[idx].add(src)
def _segment_sum(src, seg, n):
    return jax.ops.segment_sum(src, seg, n)
class _Rng:
    def __init__(self, key):
        self._k = key
    def _next(self):
        self._k, sub = jax.random.split(self._k)
        return sub
    def normal(self, shape):
        return jax.random.normal(self._next(), shape, dtype=jnp.bfloat16)
    def randint(self, lo, hi, shape):
        return jax.random.randint(self._next(), shape, lo, hi, dtype=jnp.int32)
    def uniform(self, shape, lo=0.0, hi=1.0):
        return jax.random.uniform(self._next(), shape, jnp.bfloat16, lo, hi)
    def permutation(self, n):
        return jax.random.permutation(self._next(), n)


kernel_name = 'gated_mix__linear_attn_block__swiglu_ffn__prompt'

def setup_inputs():
    _rng = _Rng(jax.random.key(int.from_bytes(__import__("os").urandom(4), "little")))
    _w = (lambda a: (lambda t: t.astype(jnp.bfloat16) if jnp.issubdtype(t.dtype, jnp.floating) else t)(jnp.asarray(a)))
    def _A_setup():
        B, S, D = 1, 2048, 512
        return {
            "x": _w((lambda *s: _rng.normal(s) * 0.05)(B, S, D)),
            "wqkv": _w((lambda *s: _rng.normal(s) * 0.8)(D, 3 * D)),
            "wo": _w((lambda *s: _rng.normal(s) * 0.05)(D, D)),
        }
    _A_in = _A_setup()

    def _B_setup():
        B, S, D, F = 1, 2048, 512, 1792
        return {
            "x": _w((lambda *s: _rng.normal(s) * 0.05)(B, S, D)),
            "w_gate": _w((lambda *s: _rng.normal(s) * 0.1)(D, F)),
            "w_up": _w((lambda *s: _rng.normal(s) * 0.1)(D, F)),
            "w_down": _w((lambda *s: _rng.normal(s) * 0.1)(F, D)),
        }
    _B_in = _B_setup()

    return {
        "A_x": _A_in["x"],
        "A_wqkv": _A_in["wqkv"],
        "A_wo": _A_in["wo"],
        "B_x": _B_in["x"],
        "B_w_gate": _B_in["w_gate"],
        "B_w_up": _B_in["w_up"],
        "B_w_down": _B_in["w_down"],
        "gate_w": _w((lambda *s: _rng.normal(s) * 0.05)(512) * 16.0),
    }

def reference(A_x, A_wqkv, A_wo, B_x, B_w_gate, B_w_up, B_w_down, gate_w):
    def _A_ref(x, wqkv, wo):
        B, S, D = x.shape
        H = 32; Dh = D // H
        qkv = (lambda x, *d: x.transpose(*d))((x @ wqkv).reshape(B, S, 3, H, Dh), 2, 0, 3, 1, 4)
        q, k, v = qkv[0], qkv[1], qkv[2]
        phi = lambda t: jnp.where(t > 0, t + 1, jnp.exp(t)) + 1e-6
        pq, pk = phi(q), phi(k)
        kv = jnp.einsum("bhsd,bhse->bhde", pk, v)
        z = jnp.einsum("bhsd->bhd", pk)
        num = jnp.einsum("bhqd,bhde->bhqe", pq, kv)
        den = jnp.einsum("bhqd,bhd->bhq", pq, z)[..., None] + 1e-6
        o = num / den
        return (lambda x, *d: x.transpose(*d))(o, 0, 2, 1, 3).reshape(B, S, D) @ wo

    def _B_ref(x, w_gate, w_up, w_down):
        g = _silu(x @ w_gate)
        u = x @ w_up
        return (g * u) @ w_down

    x = A_x
    g = _sigmoid((x * gate_w).sum(-1, keepdims=True))
    a = _A_ref(x, A_wqkv, A_wo)
    b = _B_ref(x, B_w_gate, B_w_up, B_w_down)
    return g * a + (1 - g) * b
```

```python
import functools
import jax
import jax.numpy as jnp
from jax import lax
import jax.experimental.pallas as pl
import jax.experimental.pallas.tpu as pltpu

F32 = jnp.float32
BF16 = jnp.bfloat16
U32 = jnp.uint32
HEADS = 32
LANES = 128
NT = (((1,), (1,)), ((), ()))


def _phi(t):
    return jnp.where(t > 0, t + 1.0, jnp.exp(t)) + 1e-6


def _sigmoid(t):
    return 0.5 * jnp.tanh(0.5 * t) + 0.5


def _dot(a, b):
    return jnp.dot(a, b, preferred_element_type=F32)


def build(RA=256, RB=384, CA=256, cchunks=(512, 512, 384), TQ=512, TS=640, FC=256,
          parts=(384, 192, 64), nochk=True, peel=128, prep_pos=0, layout='new', dsplit=1):
    def fn(A_x, A_wqkv, A_wo, B_x, B_w_gate, B_w_up, B_w_down, gate_w):
        B, S, D = A_x.shape
        F = B_w_gate.shape[1]
        HD = D // HEADS
        HP = HD // 2
        nf = F // FC
        ng = D // LANES
        n2 = (S - peel) // TS
        assert RA + RB + sum(cchunks) == S and sum(parts) == TS and peel + n2 * TS == S

        def kernel(x_hbm, wqkv_hbm, wo_hbm, wg_hbm, wu_hbm, wd_hbm, gw_hbm, out_hbm,
                   x_v, wq_v, wk_v, wv_v, wo_v, wg_v, wu_v, wd_v, gw_v,
                   wkT_v, tmp_v, wqTp_v, G_v, z_v, Mp_v, pq_v, zrow_v, out_v, sem):
            def cp(src, dst, i):
                return pltpu.make_async_copy(src, dst, sem.at[i])
            def x_cp(r0, n, i):
                return cp(x_hbm.at[0, pl.ds(r0, n), :], x_v.at[pl.ds(r0, n), :], i)
            c_wka = cp(wqkv_hbm.at[:, pl.ds(D, CA)], wk_v.at[:, pl.ds(0, CA)], 0)
            c_xa = x_cp(0, RA, 1)
            c_wkb = cp(wqkv_hbm.at[:, pl.ds(D + CA, D - CA)], wk_v.at[:, pl.ds(CA, D - CA)], 2)
            c_xb = x_cp(RA, RB, 2)
            c_xc = x_cp(RA + RB, S - RA - RB, 3)
            c_wq = cp(wqkv_hbm.at[:, pl.ds(0, D)], wq_v, 3)
            c_wv = cp(wqkv_hbm.at[:, pl.ds(2 * D, D)], wv_v, 4)
            c_wo = cp(wo_hbm, wo_v, 4)
            e = 4 if layout == 'new' else 6
            c_gw = cp(gw_hbm, gw_v, e)
            c_wg = cp(wg_hbm, wg_v, e)
            c_wu = cp(wu_hbm, wu_v, e)
            c_wd = cp(wd_hbm, wd_v, e)
            for c in (c_wka, c_xa, c_wkb, c_xb, c_xc, c_wq, c_wv, c_wo, c_gw, c_wg, c_wu, c_wd):
                c.start()

            def permuted(l):
                w = jnp.concatenate([tmp_v[l, pl.ds(p, HEADS, stride=HP), :] for p in range(HP)], axis=0)
                return pltpu.bitcast(w, BF16)

            def kg(r0, nr, c0, nc, first):
                xt = x_v[r0:r0 + nr, :]
                kT = lax.dot_general(wkT_v[c0:c0 + nc, :], xt, NT, preferred_element_type=F32)
                pkT = _phi(kT)
                zp = pkT[:, 0:LANES]
                for c in range(1, nr // LANES):
                    zp = zp + pkT[:, c * LANES:(c + 1) * LANES]
                g = _dot(pkT.astype(BF16), xt)
                if first:
                    G_v[c0:c0 + nc, :] = g
                    z_v[c0:c0 + nc, :] = zp
                else:
                    G_v[c0:c0 + nc, :] += g
                    z_v[c0:c0 + nc, :] += zp

            def wq_prep():
                for l in range(ng):
                    tmp_v[l] = pltpu.bitcast(wq_v[l * LANES:(l + 1) * LANES, :].T, U32)
                for l in range(ng):
                    wqTp_v[:, l * LANES:(l + 1) * LANES] = permuted(l)

            def z_prep():
                tmp_v[2 * ng] = pltpu.bitcast(z_v[...].astype(BF16), U32)
                zrow_v[...] = jnp.broadcast_to(
                    jnp.sum(permuted(2 * ng).T.astype(F32), axis=0, keepdims=True), (8, D))

            def q_all():
                for t in range(S // TQ):
                    rs = slice(t * TQ, (t + 1) * TQ)
                    pq_v[rs, :] = _phi(lax.dot_general(x_v[rs, :], wqTp_v[...], NT, preferred_element_type=F32))

            def mid():
                r = lax.broadcasted_iota(jnp.int32, (LANES, LANES), 0) // HD
                c = lax.broadcasted_iota(jnp.int32, (LANES, LANES), 1) // HD
                same = r == c
                for j in range(ng):
                    sl = slice(j * LANES, (j + 1) * LANES)
                    kv = _dot(G_v[sl, :].astype(BF16), wv_v[:, sl])
                    kv = jnp.where(same, kv, 0.0).astype(BF16)
                    m = pltpu.bitcast(_dot(kv, wo_v[sl, :]).astype(BF16), U32)
                    for l in range(ng):
                        tmp_v[ng + l, j * LANES // 2:(j + 1) * LANES // 2, :] = m[:, l * LANES:(l + 1) * LANES]
                for l in range(ng):
                    Mp_v[:, l * LANES:(l + 1) * LANES] = permuted(ng + l)

            c_wka.wait()
            wkT_v[0:CA, :] = wk_v[:, 0:CA].T
            c_xa.wait()
            kg(0, RA, 0, CA, True)
            c_wkb.wait()
            c_xb.wait()
            wkT_v[CA:D, :] = wk_v[:, CA:D].T
            kg(RA, RB, 0, CA, False)
            kg(0, RA + RB, CA, D - CA, True)
            c_xc.wait()
            c_wq.wait()
            r0 = RA + RB
            for idx, nr in enumerate(cchunks):
                if idx == prep_pos:
                    wq_prep()
                if layout == 'old' and idx == dsplit:
                    c_wv.wait()
                    c_wo.wait()
                kg(r0, nr, 0, D, False)
                r0 += nr
            if layout == 'old':
                mid()
            z_prep()
            q_all()
            if layout == 'new':
                c_wv.wait()
                c_wo.wait()
            c_gw.wait()
            c_wg.wait()
            c_wu.wait()
            c_wd.wait()
            if layout == 'new':
                mid()

            def o_copy(row, n):
                return pltpu.make_async_copy(out_v.at[pl.ds(row, n), :],
                                             out_hbm.at[0, pl.ds(row, n), :], sem.at[5])

            def rows(row, ts, prts):
                xt = x_v[pl.ds(row, ts), :]
                gw = gw_v[...].astype(F32).reshape(1, D)
                logit = jnp.sum(xt.astype(F32) * gw, axis=1, keepdims=True)
                gate = jnp.broadcast_to(_sigmoid(logit), (ts, LANES))
                og = 1.0 - gate
                pq = pq_v[pl.ds(row, ts), :]
                tz = pq * zrow_v[0:1, :]
                u = tz[:, 0:LANES]
                for j in range(1, ng):
                    u = u + tz[:, j * LANES:(j + 1) * LANES]
                sh = 2 * HEADS
                while sh < LANES:
                    u = u + pltpu.roll(u, sh, axis=1)
                    sh *= 2
                odd = (lax.broadcasted_iota(jnp.int32, (ts, LANES), 1) & 1) == 1
                den = u + jnp.where(odd, pltpu.roll(u, 1, axis=1), pltpu.roll(u, LANES - 1, axis=1))
                scale = gate / (den + 1e-6)
                pqn = jnp.concatenate(
                    [pq[:, j * LANES:(j + 1) * LANES] * scale for j in range(ng)], axis=1).astype(BF16)
                b = None
                for f in range(nf):
                    fs = slice(f * FC, (f + 1) * FC)
                    hg = _dot(xt, wg_v[:, fs])
                    hu = _dot(xt, wu_v[:, fs])
                    h = (hg * _sigmoid(hg) * hu).astype(BF16)
                    if f < nf - 1:
                        p = _dot(h, wd_v[fs, :])
                        b = p if b is None else b + p
                p0 = 0
                for pn in prts:
                    prow = row + p0
                    if not isinstance(prow, int):
                        prow = pl.multiple_of(prow, 32)
                    bp = b[p0:p0 + pn] + _dot(h[p0:p0 + pn], wd_v[fs, :])
                    a = _dot(pqn[p0:p0 + pn], Mp_v[...])
                    o = jnp.concatenate(
                        [a[:, j * LANES:(j + 1) * LANES] + og[p0:p0 + pn] * bp[:, j * LANES:(j + 1) * LANES]
                         for j in range(ng)], axis=1)
                    out_v[pl.ds(prow, pn), :] = o.astype(BF16)
                    o_copy(prow, pn).start()
                    p0 += pn

            if peel:
                rows(0, peel, (peel,))

            def tile(i, carry):
                rows(pl.multiple_of(peel + i * TS, 64), TS, parts)
                return carry

            lax.fori_loop(0, n2, tile, 0)
            o_copy(0, S).wait()

        any_spec = pl.BlockSpec(memory_space=pl.ANY)
        return pl.pallas_call(
            kernel,
            out_shape=jax.ShapeDtypeStruct((B, S, D), BF16),
            in_specs=[any_spec] * 7,
            out_specs=any_spec,
            scratch_shapes=[
                pltpu.VMEM((S, D), BF16),
                pltpu.VMEM((D, D), BF16),
                pltpu.VMEM((D, D), BF16),
                pltpu.VMEM((D, D), BF16),
                pltpu.VMEM((D, D), BF16),
                pltpu.VMEM((D, F), BF16),
                pltpu.VMEM((D, F), BF16),
                pltpu.VMEM((F, D), BF16),
                pltpu.VMEM((D,), BF16),
                pltpu.VMEM((D, D), BF16),
                pltpu.VMEM((2 * ng + 1, D // 2, LANES), U32),
                pltpu.VMEM((D, D), BF16),
                pltpu.VMEM((D, D), F32),
                pltpu.VMEM((D, LANES), F32),
                pltpu.VMEM((D, D), BF16),
                pltpu.VMEM((S, D), F32),
                pltpu.VMEM((8, D), F32),
                pltpu.VMEM((S, D), BF16),
                pltpu.SemaphoreType.DMA((7,)),
            ],
            compiler_params=pltpu.CompilerParams(vmem_limit_bytes=100 * 1024 * 1024, disable_bounds_checks=nochk,
                                                 disable_semaphore_checks=nochk),
        )(A_x, A_wqkv, A_wo, B_w_gate, B_w_up, B_w_down, gate_w)
    return fn


@jax.jit
def pallas_gated_mix__linear_attn_block__swiglu_ffn__prompt_kernel(A_x, A_wqkv, A_wo, B_x, B_w_gate, B_w_up, B_w_down, gate_w):
    return build()(A_x, A_wqkv, A_wo, B_x, B_w_gate, B_w_up, B_w_down, gate_w)
```

```python
import jax
import jax.numpy as jnp
from jax import lax
import jax.experimental.pallas as pl
import jax.experimental.pallas.tpu as pltpu

F32 = jnp.float32
BF16 = jnp.bfloat16
U32 = jnp.uint32
HEADS = 32
LANES = 128
STRIP = 16

L_TERMS = (((0, 0, 1), (1, 1, 1)), ((1, 0, 1), (1, 1, 1)), ((0, 0, 1),), ((1, 1, 1),),
           ((0, 0, 1), (0, 1, 1)), ((1, 0, 1), (0, 0, -1)), ((0, 1, 1), (1, 1, -1)))
R_TERMS = (((0, 0, 1), (1, 1, 1)), ((0, 0, 1),), ((0, 1, 1), (1, 1, -1)), ((1, 0, 1), (0, 0, -1)),
           ((1, 1, 1),), ((0, 0, 1), (0, 1, 1)), ((1, 0, 1), (1, 1, 1)))
C_TERMS = (((0, 1), (3, 1), (4, -1), (6, 1)), ((2, 1), (4, 1)), ((1, 1), (3, 1)),
           ((0, 1), (1, -1), (2, 1), (5, 1)))
X_AS_RHS = (0, 2, 6, 5, 3, 4, 1)
ORDER = (2, 4, 3, 1, 0, 6, 5)
QUADS = (1, 2, 0, 3)
ORDER_G = (2, 4, 5, 3, 0, 1, 6)
ORDER_Q = (1, 5, 4, 2, 0, 3, 6)


def _phi(t):
    return jnp.where(t > 0, t + 1.0, jnp.exp(t)) + 1e-6


def _dot(a, b):
    return jnp.dot(a, b, preferred_element_type=F32)


def _dot_nt(a, b):
    return lax.dot_general(a, b, (((1,), (1,)), ((), ())), preferred_element_type=F32)


def _combine(terms, blk):
    acc = None
    for t in terms:
        v = blk(*t[:-1])
        acc = v if acc is None else (acc + v if t[-1] > 0 else acc - v)
    return acc


def _lhs7(a11, a12, a21, a22):
    q = ((a11, a12), (a21, a22))
    return [_combine(t, lambda r, c: q[r][c]) for t in L_TERMS]


def _rhs7(b11, b12, b21, b22):
    q = ((b11, b12), (b21, b22))
    return [_combine(t, lambda r, c: q[r][c]) for t in R_TERMS]


def _out4(m):
    return [_combine(t, lambda k: m[k]) for t in C_TERMS]


def _silu_mul(c, half_scale):
    hg, hu = c[:, :LANES], c[:, LANES:]
    return hg * (half_scale * jnp.tanh(0.5 * hg) + half_scale) * hu


def _zero_after(m, r0):
    b = lax.bitcast_convert_type(m[r0:r0 + 8, 0:LANES], U32)
    return lax.bitcast_convert_type((b >> 16) >> 16, F32)


def _rep(v, nr, nc):
    v = v if nc == 1 else jnp.concatenate([v] * nc, axis=1)
    return v if nr == 1 else jnp.concatenate([v] * nr, axis=0)


def _pinned(v, pin):
    return v + _rep(pin, v.shape[0] // pin.shape[0], v.shape[1] // pin.shape[1])


@jax.jit
def pallas_gated_mix__linear_attn_block__swiglu_ffn__prompt_kernel(
    A_x: jax.Array,
    A_wqkv: jax.Array,
    A_wo: jax.Array,
    B_x: jax.Array,
    B_w_gate: jax.Array,
    B_w_up: jax.Array,
    B_w_down: jax.Array,
    gate_w: jax.Array,
):
    del B_x
    B, S, D = A_x.shape
    F = B_w_gate.shape[1]
    HD = D // HEADS
    P = S // 2
    H = D // 2
    FH = F // 2
    NPAIR = FH // H
    FL = 2 * NPAIR * LANES
    NG = D // LANES
    TS = 256
    HN = TS // 2
    NT = P // TS
    STAGES = (128, 256, 896, P)
    NS = len(STAGES)
    assert B == 1 and H == 2 * LANES and FH == FL + LANES and P % TS == 0 and HD == 16

    def kernel(x_hbm, wqkv_hbm, wo_hbm, wg_hbm, wu_hbm, wd_hbm, gw_hbm, out_hbm,
               x_v, wq_v, wk_v, wv_v, wo_v, wg_v, wu_v, wd_v, gw_v,
               t1_v, t2_v, sk_v, g1_v, d1_v, g2_v, d2_v,
               gm_v, z_v, tmp_v, q_v, row_v, h1_v, h_v, pn_v, cg_v, out_v, sem):
        SEM_W, SEM_O = NS + 1, NS + 2
        groups = [[] for _ in range(NS + 2)]

        def fetch(src, dst, g):
            d = pltpu.make_async_copy(src, dst, sem.at[g])
            groups[g].append(d)
            d.start()

        for s, r in enumerate(STAGES):
            r0 = STAGES[s - 1] if s else 0
            if s < 2:
                fetch(wqkv_hbm.at[:, pl.ds(D + s * H, H)], wk_v.at[:, pl.ds(s * H, H)], 2 * s)
            fetch(x_hbm.at[:, pl.ds(r0, r - r0), :], x_v.at[:, pl.ds(r0, r - r0), :], s + 1)
        fetch(gw_hbm, gw_v, NS)
        fetch(wqkv_hbm.at[:, pl.ds(0, D)], wq_v, NS)
        fetch(wg_hbm, wg_v, NS)
        fetch(wu_hbm, wu_v, NS)
        fetch(wd_hbm, wd_v, SEM_W)
        fetch(wqkv_hbm.at[:, pl.ds(2 * D, D)], wv_v, SEM_W)
        fetch(wo_hbm, wo_v, SEM_W)

        def wait_group(g):
            for d in groups[g]:
                d.wait()

        def at(row, off, n):
            r = row + off
            return pl.ds(r if isinstance(r, int) else pl.multiple_of(r, STRIP), n)

        def load2(ref, k, r0, n):
            return jnp.concatenate([ref[2 * k + l, r0:r0 + n, :] for l in range(2)], axis=1)

        def store2(ref, k, r0, v):
            for l in range(2):
                ref[2 * k + l, r0:r0 + v.shape[0], :] = v[:, l * LANES:(l + 1) * LANES].astype(BF16)

        jobs = []
        clock = dict(t=0.0, start=0.0, rate=0.0, done=0)

        def plan(total, skip_head, skip_tail):
            clock.update(t=0.0, start=skip_head, done=0, rate=len(jobs) / (total - skip_head - skip_tail))

        def run_jobs(m, k, weight=1.0):
            per8 = weight * 2 * (k // LANES) * (m.shape[1] // LANES)
            for r0 in range(0, m.shape[0], 8):
                clock['t'] += per8
                while jobs and clock['done'] < (clock['t'] - clock['start']) * clock['rate']:
                    clock['done'] += 1
                    jobs.pop(0)(_zero_after(m, r0))

        def x_op(i, row, n):
            if len(L_TERMS[i]) == 1:
                r, c, _ = L_TERMS[i][0]
                return x_v[r, row:row + n, c * H:(c + 1) * H]
            return load2(t1_v, i, row, n)

        def x_prep(p0, n):
            top = x_v[0, p0:p0 + n, :].astype(F32)
            bot = x_v[1, p0:p0 + n, :].astype(F32)
            t = _lhs7(top[:, :H], top[:, H:], bot[:, :H], bot[:, H:])
            for i in ORDER:
                if len(L_TERMS[i]) > 1:
                    store2(t1_v, i, p0, t[i])
            return [t[i].astype(BF16) if len(L_TERMS[i]) > 1 else x_op(i, p0, n) for i in range(7)]

        def wk_prep(grp):
            wt = wk_v[:, grp * H:(grp + 1) * H].T.astype(F32)
            r = _rhs7(wt[:LANES, :H], wt[LANES:, :H], wt[:LANES, H:], wt[LANES:, H:])
            for i in ORDER:
                store2(sk_v, i, grp * LANES, r[i])

        def kg(p0, g0, g1, first, new_rows):
            n = LANES
            xs = x_prep(p0, n) if new_rows else [x_op(i, p0, n) for i in range(7)]
            m = [None] * 7
            for i in ORDER:
                m[i] = _dot_nt(load2(sk_v, i, g0 * LANES, (g1 - g0) * LANES), xs[i])
                run_jobs(m[i], H)
            c11, c12, c21, c22 = [_phi(c) for c in _out4(m)]
            for half, zp in enumerate((c11 + c21, c12 + c22)):
                for g in range(g0, g1):
                    zs = slice((2 * g + half) * LANES, (2 * g + half + 1) * LANES)
                    zz = zp[(g - g0) * LANES:(g - g0 + 1) * LANES]
                    if first:
                        z_v[zs, :] = zz
                    else:
                        z_v[zs, :] += zz
            a = _lhs7(c11, c21, c12, c22)
            for i in ORDER_G:
                gm = _dot(a[i].astype(BF16), xs[X_AS_RHS[i]])
                run_jobs(gm, n)
                if first:
                    gm_v[i, g0 * LANES:g1 * LANES, :] = gm
                else:
                    gm_v[i, g0 * LANES:g1 * LANES, :] += gm

        def perm_store(w, slab0):
            nl = w.shape[1] // LANES
            w = w.reshape(HEADS, 2, HD // 2, w.shape[1])
            for b in range(2):
                wh = w[:, b].reshape(H, -1)
                for l in range(nl):
                    tmp_v[slab0 + b * nl + l, 0:H, :] = wh[:, l * LANES:(l + 1) * LANES]

        def perm_load(slab, k0=0, n=H):
            hr, g = HD // 2, min(n, HEADS)
            return jnp.concatenate([tmp_v[slab, pl.ds((k % HEADS) * hr + k // HEADS, g, stride=hr), :]
                                    for k in range(k0, k0 + n, g)], axis=0)

        def permuted(w, slab0):
            nl = w.shape[1] // LANES
            perm_store(w, slab0)
            return [jnp.concatenate([perm_load(slab0 + b * nl + l) for l in range(nl)], axis=1) for b in range(2)]

        def rows_prep():
            zp = jnp.concatenate(permuted(z_v[...], 4 * NG), axis=0)
            row_v[0:8, :] = jnp.broadcast_to(jnp.sum(zp.T, axis=0, keepdims=True), (8, D))
            row_v[8:16, :] = jnp.broadcast_to(gw_v[...].astype(F32).reshape(1, D), (8, D))

        def one_level_job(blk, dst, r0):
            def job(pin):
                r = _rhs7(_pinned(blk(0, 0), pin), blk(0, 1), blk(1, 0), _pinned(blk(1, 1), pin))
                for i in range(7):
                    store2(dst, i, r0, r[i])
            return job

        def two_level_jobs(blk, dst, slab, r0, terms):
            def make(i):
                def job(pin):
                    pin = _rep(pin, STRIP // 8, 2)
                    q = [_combine(terms[i], lambda R, C: _pinned(blk(R, C, r).astype(F32), pin)
                                  if (R, C) == terms[i][0][:2] else blk(R, C, r).astype(F32)) for r in range(2)]
                    q = [[q[r][:, c * LANES:(c + 1) * LANES] for c in range(2)] for r in range(2)]
                    for j in range(7):
                        dst[slab(7 * i + j), r0:r0 + STRIP, :] = _combine(
                            terms[j], lambda r, c: q[r][c]).astype(BF16)
                return job
            jobs.extend(make(i) for i in (X_AS_RHS if terms is L_TERMS else range(7)))

        def gate_up_weight_jobs():
            for k0 in range(0, H, STRIP):
                jobs.append(one_level_job(lambda r, c, k0=k0: jnp.concatenate(
                    [w_v[r * H + k0:r * H + k0 + STRIP, c * FH + FL:c * FH + FL + LANES].astype(F32)
                     for w_v in (wg_v, wu_v)], axis=1), g1_v, k0))
            for p in range(NPAIR):
                for wi, w_v in enumerate((wg_v, wu_v)):
                    for k0 in range(0, LANES, STRIP):
                        two_level_jobs(
                            lambda R, C, r, w_v=w_v, p=p, k0=k0: w_v[
                                R * H + r * LANES + k0:R * H + r * LANES + k0 + STRIP,
                                C * FH + p * H:C * FH + (p + 1) * H],
                            g2_v, lambda ij, p=p, wi=wi: 2 * (49 * p + ij) + wi, k0, R_TERMS)

        def down_weight_jobs():
            for p in range(NPAIR):
                for k0 in range(0, LANES, STRIP):
                    two_level_jobs(
                        lambda R, C, r, k0=p * H + k0: wd_v[
                            R * FH + r * LANES + k0:R * FH + r * LANES + k0 + STRIP, C * H:(C + 1) * H],
                        d2_v, lambda ij: ij, p * LANES + k0, R_TERMS)
            for k0 in range(0, LANES, STRIP):
                jobs.append(one_level_job(lambda r, c, k0=k0: wd_v[
                    r * FH + FL + k0:r * FH + FL + k0 + STRIP, c * H:(c + 1) * H].astype(F32), d1_v, k0))

        def x_tile_jobs(row):
            for k0 in range(0, HN, STRIP):
                rows = [at(row, r * HN + k0, STRIP) for r in range(2)]
                two_level_jobs(lambda R, C, r, rows=rows: x_v[R, rows[r], C * H:(C + 1) * H],
                               t2_v, lambda ij: ij, k0, L_TERMS)

        def gate_jobs(row):
            def make(hf, r0):
                def job(pin):
                    gw = _rep(_pinned(row_v[8:16, :], pin), STRIP // 8, 1)
                    logit = jnp.sum(x_v[hf, at(row, r0, STRIP), :].astype(F32) * gw, axis=1, keepdims=True)
                    cg_v[hf, r0:r0 + STRIP, :] = jnp.broadcast_to(
                        0.25 - 0.25 * jnp.tanh(0.5 * logit), (STRIP, LANES))
                return job
            jobs.extend(make(hf, r0) for hf in range(2) for r0 in range(0, TS, STRIP))

        def attn_jobs(row, zero):
            def make(hf, r0):
                def job(pin):
                    rr = at(row, r0, STRIP)
                    og = 2.0 * cg_v[hf, r0:r0 + STRIP, :]
                    if hf == 0:
                        m5 = _pinned(q_v[4, rr, :], pin)
                        q = [q_v[0, rr, :] - m5 + q_v[3, rr, :] + q_v[6, rr, :], q_v[2, rr, :] + m5]
                    else:
                        m2 = _pinned(q_v[1, rr, :], pin)
                        q = [m2 + q_v[3, rr, :], q_v[0, rr, :] - m2 + q_v[2, rr, :] + q_v[5, rr, :]]
                    pq = _phi(jnp.concatenate(q, axis=1))
                    pz = pq * _rep(row_v[0:8, :], STRIP // 8, 1)
                    den = pz[:, 0:LANES]
                    for j in range(1, NG):
                        den = den + pz[:, j * LANES:(j + 1) * LANES]
                    den = den + pltpu.roll(den, HEADS, axis=1)
                    den = den + pltpu.roll(den, 2 * HEADS, axis=1)
                    scale = _rep((1.0 - og) / (den + 1e-6), 1, 2)
                    pn_v[hf + zero, r0:r0 + STRIP, :] = jnp.concatenate(
                        [h1_v[hf, rr, 0:LANES] * og, pq[:, :H] * scale,
                         h1_v[hf, rr, LANES:2 * LANES] * og, pq[:, H:] * scale], axis=1)
                return job
            jobs.extend(make(hf, r0) for hf in range(2) for r0 in range(0, TS, STRIP))

        kvs = []

        def state_kv():
            g11, g12, g21, g22 = _out4([gm_v[i] for i in range(7)])
            r = lax.broadcasted_iota(jnp.int32, (LANES, LANES), 0) // HD
            c = lax.broadcasted_iota(jnp.int32, (LANES, LANES), 1) // HD
            for j in range(NG):
                gs = slice((j // 2) * LANES, (j // 2 + 1) * LANES)
                gl, gr = (g11, g12) if j % 2 == 0 else (g21, g22)
                gj = jnp.concatenate([gl[gs], gr[gs]], axis=1).astype(BF16)
                kv = _dot(gj, wv_v[:, j * LANES:(j + 1) * LANES])
                kvs.append(jnp.where(r == c, kv, 0.0).astype(BF16))

        def state_m():
            perm_store(jnp.concatenate([_dot(kvs[j], wo_v[j * LANES:(j + 1) * LANES, :]) for j in range(NG)],
                                       axis=0), 2 * NG)
            del jobs[-(H // STRIP):]
            for n, k0 in enumerate(range(0, H, STRIP)):
                jobs.insert(10 + 3 * n, one_level_job(lambda r, c, k0=k0: jnp.concatenate(
                    [perm_load((2 + r) * NG + 2 * c + l, k0, STRIP) for l in range(2)], axis=1), d1_v, LANES + k0))

        def odd_chunk(t, hooks):
            m = [None] * 7
            for k, i in enumerate(ORDER):
                if k in hooks:
                    hooks[k]()
                m[i] = _dot(x_op(i, t * TS, TS), load2(g1_v, i, 0, H))
                run_jobs(m[i], H)
            for q, c in enumerate(_out4(m)):
                h1_v[q // 2, t * TS:(t + 1) * TS, (q % 2) * LANES:(q % 2 + 1) * LANES] = _silu_mul(c, 0.5)

        def prologue():
            wait_group(0)
            wk_prep(0)
            wait_group(1)
            for p0 in range(0, STAGES[0], LANES):
                kg(p0, 0, 1, p0 == 0, True)
            wait_group(2)
            wk_prep(1)
            for p0 in range(STAGES[0], STAGES[1], LANES):
                kg(p0, 0, 1, False, True)
            for p0 in range(0, STAGES[1], LANES):
                kg(p0, 1, 2, p0 == 0, False)
            wait_group(3)
            for p0 in range(STAGES[1], STAGES[2], LANES):
                kg(p0, 0, 2, False, True)

            wait_group(4)
            n1, n2 = permuted(wq_v[...].T.astype(F32), 0)
            sq = [u.astype(BF16) for u in _rhs7(n1[:, :H], n2[:, :H], n1[:, H:], n2[:, H:])]
            gate_up_weight_jobs()
            plan(14 * (P - STAGES[2]) + 7 * P, 14 * (P - STAGES[2]), 300)
            for p0 in range(STAGES[2], P, LANES):
                kg(p0, 0, 2, False, True)
            rows_prep()
            for i in ORDER_Q:
                m = _dot_nt(x_op(i, 0, P), sq[i])
                run_jobs(m, H)
                q_v[i] = m
            assert not jobs

            wait_group(SEM_W)
            gate_jobs(0)
            x_tile_jobs(0)
            down_weight_jobs()
            jobs.extend([None] * (H // STRIP))
            plan(7 * P, 0, 300)
            for t in range(NT):
                odd_chunk(t, {2: state_kv, 5: state_m} if t == 0 else {})
            assert not jobs

        def gate_up(row, zero):
            light_outer, light_inner = (0, 2, 4), (1, 2, 3, 4, 5, 6)
            attn_jobs(row, zero)
            plan(NPAIR * len(light_outer) * len(light_inner) * HN // 2, 0, 1)
            for p in range(NPAIR):
                mo = [None] * 7
                for ko, i in enumerate(ORDER):
                    m = [None] * 7
                    for ki, j in enumerate(ORDER):
                        m[j] = _dot(t2_v[7 * i + j], load2(g2_v, 49 * p + 7 * i + j, 0, LANES))
                        if ko in light_outer and ki in light_inner:
                            run_jobs(m[j], LANES)
                    mo[i] = _out4(m)
                c16 = [_out4([mo[i][inner] for i in range(7)]) for inner in range(4)]
                for q in QUADS:
                    for inner in QUADS:
                        r, c = divmod(inner, 2)
                        c0 = (q % 2) * FL + p * H + c * LANES
                        h_v[q // 2, at(row, r * HN, HN), c0:c0 + LANES] = _silu_mul(
                            c16[inner][q], cg_v[q // 2, r * HN:(r + 1) * HN, :])
            assert not jobs

        def emit(hf, rows, c0, cn):
            pltpu.make_async_copy(out_v.at[hf, rows, pl.ds(c0, cn)], out_hbm.at[hf, rows, pl.ds(c0, cn)],
                                  sem.at[SEM_O]).start()

        def down(row, nxt):
            K1 = LANES + H
            AHEAD, WEIGHT = 3, 4.0

            def hblk(R, C, r, c):
                return jnp.concatenate(
                    [h_v[R, at(row, r * HN, HN), C * FL + p * H + c * LANES:C * FL + p * H + (c + 1) * LANES]
                     for p in range(NPAIR)], axis=1)
            v = [u.astype(BF16) for u in _lhs7(*[pn_v[R, :, C * K1:(C + 1) * K1] for R in range(2) for C in range(2)])]
            x_tile_jobs(nxt)
            gate_jobs(nxt)
            plan(49 * NPAIR * HN // 4 + WEIGHT * 7 * 6 * TS // 4, 300, 400)
            m1 = [None] * 7

            def one_level(k):
                if k < 7:
                    m1[ORDER[k]] = _dot(v[ORDER[k]], load2(d1_v, ORDER[k], 0, K1))
                    run_jobs(m1[ORDER[k]], K1, WEIGHT)
            for k in range(AHEAD - 1):
                one_level(k)
            mo = [None] * 7
            done = set()
            for ko, i in enumerate(ORDER):
                one_level(AHEAD - 1 + ko)
                a = _lhs7(*[_combine(L_TERMS[i], lambda R, C: hblk(R, C, r, c)) for r in range(2) for c in range(2)])
                m = [None] * 7
                for j in ORDER:
                    m[j] = _dot(a[j].astype(BF16), d2_v[7 * i + j])
                    run_jobs(m[j], NPAIR * LANES)
                mo[i] = [c + m1[i][(k // 2) * HN:(k // 2 + 1) * HN, (k % 2) * LANES:(k % 2 + 1) * LANES]
                         for k, c in enumerate(_out4(m))]
                for q in QUADS:
                    if q in done or any(mo[t[0]] is None for t in C_TERMS[q]):
                        continue
                    done.add(q)
                    o = [_combine(C_TERMS[q], lambda kk: mo[kk][k]) for k in range(4)]
                    c0 = (q % 2) * H
                    if q == QUADS[-1]:
                        for k in QUADS:
                            rows, c1 = at(row, (k // 2) * HN, HN), c0 + (k % 2) * LANES
                            out_v[q // 2, rows, c1:c1 + LANES] = o[k].astype(BF16)
                            emit(q // 2, rows, c1, LANES)
                    else:
                        for r in range(2):
                            out_v[q // 2, at(row, r * HN, HN), c0:c0 + H] = jnp.concatenate(
                                o[2 * r:2 * r + 2], axis=1).astype(BF16)
                        emit(q // 2, at(row, 0, TS), c0, H)
            assert not jobs

        def tile(i, carry):
            pl.when(i == 0)(prologue)
            row = pl.multiple_of(i * TS, TS)
            gate_up(row, i // NT)
            down(row, pl.multiple_of(jnp.minimum(i + 1, NT - 1) * TS, TS))
            return carry

        lax.fori_loop(0, NT, tile, 0)
        pltpu.make_async_copy(out_v, out_hbm, sem.at[SEM_O]).wait()

    any_spec = pl.BlockSpec(memory_space=pl.ANY)
    out = pl.pallas_call(
        kernel,
        out_shape=jax.ShapeDtypeStruct((2, P, D), BF16),
        in_specs=[any_spec] * 7,
        out_specs=any_spec,
        scratch_shapes=[
            pltpu.VMEM((2, P, D), BF16),
            pltpu.VMEM((D, D), BF16),
            pltpu.VMEM((D, D), BF16),
            pltpu.VMEM((D, D), BF16),
            pltpu.VMEM((D, D), BF16),
            pltpu.VMEM((D, F), BF16),
            pltpu.VMEM((D, F), BF16),
            pltpu.VMEM((F, D), BF16),
            pltpu.VMEM((D,), BF16),
            pltpu.VMEM((14, P, LANES), BF16),
            pltpu.VMEM((49, HN, LANES), BF16),
            pltpu.VMEM((14, H, LANES), BF16),
            pltpu.VMEM((14, H, LANES), BF16),
            pltpu.VMEM((14, LANES + H, LANES), BF16),
            pltpu.VMEM((NPAIR * 49 * 2, LANES, LANES), BF16),
            pltpu.VMEM((49, NPAIR * LANES, LANES), BF16),
            pltpu.VMEM((7, H, H), F32),
            pltpu.VMEM((D, LANES), F32),
            pltpu.VMEM((4 * NG + 2, H + 32, LANES), F32),
            pltpu.VMEM((7, P, H), F32),
            pltpu.VMEM((16, D), F32),
            pltpu.VMEM((2, P, 2 * LANES), F32),
            pltpu.VMEM((2, P, 2 * FL), F32),
            pltpu.VMEM((2, TS, 2 * (LANES + H)), F32),
            pltpu.VMEM((2, TS, LANES), F32),
            pltpu.VMEM((2, P, D), BF16),
            pltpu.SemaphoreType.DMA((NS + 3,)),
        ],
        compiler_params=pltpu.CompilerParams(
            vmem_limit_bytes=110 * 1024 * 1024,
            disable_bounds_checks=True,
            disable_semaphore_checks=True,
        ),
    )(A_x.reshape(2, P, D), A_wqkv, A_wo, B_w_gate, B_w_up, B_w_down, gate_w)
    return out.reshape(B, S, D)
```

```python
import jax
import jax.numpy as jnp
from jax import lax
import jax.experimental.pallas as pl
import jax.experimental.pallas.tpu as pltpu

F32 = jnp.float32
BF16 = jnp.bfloat16
U32 = jnp.uint32
HEADS = 32
LANES = 128
STRIP = 16

L_TERMS = (((0, 0, 1), (1, 1, 1)), ((1, 0, 1), (1, 1, 1)), ((0, 0, 1),), ((1, 1, 1),),
           ((0, 0, 1), (0, 1, 1)), ((1, 0, 1), (0, 0, -1)), ((0, 1, 1), (1, 1, -1)))
R_TERMS = (((0, 0, 1), (1, 1, 1)), ((0, 0, 1),), ((0, 1, 1), (1, 1, -1)), ((1, 0, 1), (0, 0, -1)),
           ((1, 1, 1),), ((0, 0, 1), (0, 1, 1)), ((1, 0, 1), (1, 1, 1)))
C_TERMS = (((0, 1), (3, 1), (4, -1), (6, 1)), ((2, 1), (4, 1)), ((1, 1), (3, 1)),
           ((0, 1), (1, -1), (2, 1), (5, 1)))
X_AS_RHS = (0, 2, 6, 5, 3, 4, 1)
ORDER = (2, 4, 3, 1, 0, 6, 5)
QUADS = (1, 2, 0, 3)
ORDER_G = (2, 4, 5, 3, 0, 1, 6)
ORDER_Q = (1, 5, 4, 2, 0, 3, 6)


def _phi(t):
    return jnp.where(t > 0, t + 1.0, jnp.exp(t)) + 1e-6


def _dot(a, b):
    return jnp.dot(a, b, preferred_element_type=F32)


def _dot_nt(a, b):
    return lax.dot_general(a, b, (((1,), (1,)), ((), ())), preferred_element_type=F32)


def _combine(terms, blk):
    acc = None
    for t in terms:
        v = blk(*t[:-1])
        acc = v if acc is None else (acc + v if t[-1] > 0 else acc - v)
    return acc


def _lhs7(a11, a12, a21, a22):
    q = ((a11, a12), (a21, a22))
    return [_combine(t, lambda r, c: q[r][c]) for t in L_TERMS]


def _rhs7(b11, b12, b21, b22):
    q = ((b11, b12), (b21, b22))
    return [_combine(t, lambda r, c: q[r][c]) for t in R_TERMS]


def _out4(m):
    return [_combine(t, lambda k: m[k]) for t in C_TERMS]


def _silu_mul(c, half_scale):
    hg, hu = c[:, :LANES], c[:, LANES:]
    return hg * (half_scale * jnp.tanh(0.5 * hg) + half_scale) * hu


def _zero_after(m, r0):
    b = lax.bitcast_convert_type(m[r0:r0 + 8, 0:LANES], U32)
    return lax.bitcast_convert_type((b >> 16) >> 16, F32)


def _rep(v, nr, nc):
    v = v if nc == 1 else jnp.concatenate([v] * nc, axis=1)
    return v if nr == 1 else jnp.concatenate([v] * nr, axis=0)


def _pinned(v, pin):
    return v + _rep(pin, v.shape[0] // pin.shape[0], v.shape[1] // pin.shape[1])


@jax.jit
def pallas_gated_mix__linear_attn_block__swiglu_ffn__prompt_kernel(
    A_x: jax.Array,
    A_wqkv: jax.Array,
    A_wo: jax.Array,
    B_x: jax.Array,
    B_w_gate: jax.Array,
    B_w_up: jax.Array,
    B_w_down: jax.Array,
    gate_w: jax.Array,
):
    del B_x
    B, S, D = A_x.shape
    F = B_w_gate.shape[1]
    HD = D // HEADS
    P = S // 2
    H = D // 2
    FH = F // 2
    NPAIR = FH // H
    FL = 2 * NPAIR * LANES
    NG = D // LANES
    TS = 256
    HN = TS // 2
    NT = P // TS
    STAGES = (128, 256, 896, P)
    NS = len(STAGES)
    assert B == 1 and H == 2 * LANES and FH == FL + LANES and P % TS == 0 and HD == 16

    def kernel(x_hbm, wqkv_hbm, wo_hbm, wg_hbm, wu_hbm, wd_hbm, gw_hbm, out_hbm,
               x_v, wq_v, wk_v, wv_v, wo_v, wg_v, wu_v, wd_v, gw_v,
               t1_v, t2_v, sk_v, g1_v, d1_v, g2_v, d2_v,
               gm_v, z_v, tmp_v, q_v, row_v, h1_v, h_v, pn_v, cg_v, out_v, sem):
        SEM_W, SEM_O = NS + 1, NS + 2
        groups = [[] for _ in range(NS + 2)]

        def fetch(src, dst, g):
            d = pltpu.make_async_copy(src, dst, sem.at[g])
            groups[g].append(d)
            d.start()

        for s, r in enumerate(STAGES):
            r0 = STAGES[s - 1] if s else 0
            if s < 2:
                fetch(wqkv_hbm.at[:, pl.ds(D + s * H, H)], wk_v.at[:, pl.ds(s * H, H)], 2 * s)
            fetch(x_hbm.at[:, pl.ds(r0, r - r0), :], x_v.at[:, pl.ds(r0, r - r0), :], s + 1)
        fetch(gw_hbm, gw_v, NS)
        fetch(wqkv_hbm.at[:, pl.ds(0, D)], wq_v, NS)
        fetch(wg_hbm, wg_v, NS)
        fetch(wu_hbm, wu_v, NS)
        fetch(wd_hbm, wd_v, SEM_W)
        fetch(wqkv_hbm.at[:, pl.ds(2 * D, D)], wv_v, SEM_W)
        fetch(wo_hbm, wo_v, SEM_W)

        def wait_group(g):
            for d in groups[g]:
                d.wait()

        def at(row, off, n):
            r = row + off
            return pl.ds(r if isinstance(r, int) else pl.multiple_of(r, STRIP), n)

        def load2(ref, k, r0, n):
            return jnp.concatenate([ref[2 * k + l, r0:r0 + n, :] for l in range(2)], axis=1)

        def store2(ref, k, r0, v):
            for l in range(2):
                ref[2 * k + l, r0:r0 + v.shape[0], :] = v[:, l * LANES:(l + 1) * LANES].astype(BF16)

        jobs = []
        clock = dict(t=0.0, start=0.0, rate=0.0, done=0)

        def plan(total, skip_head, skip_tail):
            clock.update(t=0.0, start=skip_head, done=0, rate=len(jobs) / (total - skip_head - skip_tail))

        def run_jobs(m, k, weight=1.0):
            per8 = weight * 2 * (k // LANES) * (m.shape[1] // LANES)
            for r0 in range(0, m.shape[0], 8):
                clock['t'] += per8
                while jobs and clock['done'] < (clock['t'] - clock['start']) * clock['rate']:
                    clock['done'] += 1
                    jobs.pop(0)(_zero_after(m, r0))

        def x_op(i, row, n):
            if len(L_TERMS[i]) == 1:
                r, c, _ = L_TERMS[i][0]
                return x_v[r, row:row + n, c * H:(c + 1) * H]
            return load2(t1_v, i, row, n)

        def x_prep(p0, n):
            top = x_v[0, p0:p0 + n, :].astype(F32)
            bot = x_v[1, p0:p0 + n, :].astype(F32)
            t = _lhs7(top[:, :H], top[:, H:], bot[:, :H], bot[:, H:])
            for i in ORDER:
                if len(L_TERMS[i]) > 1:
                    store2(t1_v, i, p0, t[i])
            return [t[i].astype(BF16) if len(L_TERMS[i]) > 1 else x_op(i, p0, n) for i in range(7)]

        def wk_prep(grp):
            wt = wk_v[:, grp * H:(grp + 1) * H].T.astype(F32)
            r = _rhs7(wt[:LANES, :H], wt[LANES:, :H], wt[:LANES, H:], wt[LANES:, H:])
            for i in ORDER:
                store2(sk_v, i, grp * LANES, r[i])

        def kg(p0, g0, g1, first, new_rows):
            n = LANES
            xs = x_prep(p0, n) if new_rows else [x_op(i, p0, n) for i in range(7)]
            m = [None] * 7
            for i in ORDER:
                m[i] = _dot_nt(load2(sk_v, i, g0 * LANES, (g1 - g0) * LANES), xs[i])
                run_jobs(m[i], H)
            c11, c12, c21, c22 = [_phi(c) for c in _out4(m)]
            for half, zp in enumerate((c11 + c21, c12 + c22)):
                for g in range(g0, g1):
                    zs = slice((2 * g + half) * LANES, (2 * g + half + 1) * LANES)
                    zz = zp[(g - g0) * LANES:(g - g0 + 1) * LANES]
                    if first:
                        z_v[zs, :] = zz
                    else:
                        z_v[zs, :] += zz
            a = _lhs7(c11, c21, c12, c22)
            for i in ORDER_G:
                gm = _dot(a[i].astype(BF16), xs[X_AS_RHS[i]])
                run_jobs(gm, n)
                if first:
                    gm_v[i, g0 * LANES:g1 * LANES, :] = gm
                else:
                    gm_v[i, g0 * LANES:g1 * LANES, :] += gm

        def perm_store(w, slab0):
            nl = w.shape[1] // LANES
            w = w.reshape(HEADS, 2, HD // 2, w.shape[1])
            for b in range(2):
                wh = w[:, b].reshape(H, -1)
                for l in range(nl):
                    tmp_v[slab0 + b * nl + l, 0:H, :] = wh[:, l * LANES:(l + 1) * LANES]

        def perm_load(slab, k0=0, n=H):
            hr, g = HD // 2, min(n, HEADS)
            return jnp.concatenate([tmp_v[slab, pl.ds((k % HEADS) * hr + k // HEADS, g, stride=hr), :]
                                    for k in range(k0, k0 + n, g)], axis=0)

        def permuted(w, slab0):
            nl = w.shape[1] // LANES
            perm_store(w, slab0)
            return [jnp.concatenate([perm_load(slab0 + b * nl + l) for l in range(nl)], axis=1) for b in range(2)]

        def rows_prep():
            zp = jnp.concatenate(permuted(z_v[...], 4 * NG), axis=0)
            row_v[0:8, :] = jnp.broadcast_to(jnp.sum(zp.T, axis=0, keepdims=True), (8, D))
            row_v[8:16, :] = jnp.broadcast_to(gw_v[...].astype(F32).reshape(1, D), (8, D))

        def one_level_job(blk, dst, r0):
            def job(pin):
                r = _rhs7(_pinned(blk(0, 0), pin), blk(0, 1), blk(1, 0), _pinned(blk(1, 1), pin))
                for i in range(7):
                    store2(dst, i, r0, r[i])
            return job

        def two_level_jobs(blk, dst, slab, r0, terms):
            def make(i):
                def job(pin):
                    pin = _rep(pin, STRIP // 8, 2)
                    q = [_combine(terms[i], lambda R, C: _pinned(blk(R, C, r).astype(F32), pin)
                                  if (R, C) == terms[i][0][:2] else blk(R, C, r).astype(F32)) for r in range(2)]
                    q = [[q[r][:, c * LANES:(c + 1) * LANES] for c in range(2)] for r in range(2)]
                    for j in range(7):
                        dst[slab(7 * i + j), r0:r0 + STRIP, :] = _combine(
                            terms[j], lambda r, c: q[r][c]).astype(BF16)
                return job
            jobs.extend(make(i) for i in (X_AS_RHS if terms is L_TERMS else range(7)))

        def gate_up_weight_jobs():
            for k0 in range(0, H, STRIP):
                jobs.append(one_level_job(lambda r, c, k0=k0: jnp.concatenate(
                    [w_v[r * H + k0:r * H + k0 + STRIP, c * FH + FL:c * FH + FL + LANES].astype(F32)
                     for w_v in (wg_v, wu_v)], axis=1), g1_v, k0))
            for p in range(NPAIR):
                for wi, w_v in enumerate((wg_v, wu_v)):
                    for k0 in range(0, LANES, STRIP):
                        two_level_jobs(
                            lambda R, C, r, w_v=w_v, p=p, k0=k0: w_v[
                                R * H + r * LANES + k0:R * H + r * LANES + k0 + STRIP,
                                C * FH + p * H:C * FH + (p + 1) * H],
                            g2_v, lambda ij, p=p, wi=wi: 2 * (49 * p + ij) + wi, k0, R_TERMS)

        def down_weight_jobs():
            for p in range(NPAIR):
                for k0 in range(0, LANES, STRIP):
                    two_level_jobs(
                        lambda R, C, r, k0=p * H + k0: wd_v[
                            R * FH + r * LANES + k0:R * FH + r * LANES + k0 + STRIP, C * H:(C + 1) * H],
                        d2_v, lambda ij: ij, p * LANES + k0, R_TERMS)
            for k0 in range(0, LANES, STRIP):
                jobs.append(one_level_job(lambda r, c, k0=k0: wd_v[
                    r * FH + FL + k0:r * FH + FL + k0 + STRIP, c * H:(c + 1) * H].astype(F32), d1_v, k0))

        def x_tile_jobs(row):
            for k0 in range(0, HN, STRIP):
                rows = [at(row, r * HN + k0, STRIP) for r in range(2)]
                two_level_jobs(lambda R, C, r, rows=rows: x_v[R, rows[r], C * H:(C + 1) * H],
                               t2_v, lambda ij: ij, k0, L_TERMS)

        def gate_jobs(row):
            def make(hf, r0):
                def job(pin):
                    gw = _rep(_pinned(row_v[8:16, :], pin), STRIP // 8, 1)
                    logit = jnp.sum(x_v[hf, at(row, r0, STRIP), :].astype(F32) * gw, axis=1, keepdims=True)
                    cg_v[hf, r0:r0 + STRIP, :] = jnp.broadcast_to(
                        0.25 - 0.25 * jnp.tanh(0.5 * logit), (STRIP, LANES))
                return job
            jobs.extend(make(hf, r0) for hf in range(2) for r0 in range(0, TS, STRIP))

        def attn_jobs(row, zero):
            def make(hf, r0):
                def job(pin):
                    rr = at(row, r0, STRIP)
                    og = 2.0 * cg_v[hf, r0:r0 + STRIP, :]
                    if hf == 0:
                        m5 = _pinned(q_v[4, rr, :], pin)
                        q = [q_v[0, rr, :] - m5 + q_v[3, rr, :] + q_v[6, rr, :], q_v[2, rr, :] + m5]
                    else:
                        m2 = _pinned(q_v[1, rr, :], pin)
                        q = [m2 + q_v[3, rr, :], q_v[0, rr, :] - m2 + q_v[2, rr, :] + q_v[5, rr, :]]
                    pq = _phi(jnp.concatenate(q, axis=1))
                    pz = pq * _rep(row_v[0:8, :], STRIP // 8, 1)
                    den = pz[:, 0:LANES]
                    for j in range(1, NG):
                        den = den + pz[:, j * LANES:(j + 1) * LANES]
                    den = den + pltpu.roll(den, HEADS, axis=1)
                    den = den + pltpu.roll(den, 2 * HEADS, axis=1)
                    scale = _rep((1.0 - og) / (den + 1e-6), 1, 2)
                    pn_v[hf + zero, r0:r0 + STRIP, :] = jnp.concatenate(
                        [h1_v[hf, rr, 0:LANES] * og, pq[:, :H] * scale,
                         h1_v[hf, rr, LANES:2 * LANES] * og, pq[:, H:] * scale], axis=1)
                return job
            jobs.extend(make(hf, r0) for hf in range(2) for r0 in range(0, TS, STRIP))

        kvs = []

        def state_kv():
            g11, g12, g21, g22 = _out4([gm_v[i] for i in range(7)])
            r = lax.broadcasted_iota(jnp.int32, (LANES, LANES), 0) // HD
            c = lax.broadcasted_iota(jnp.int32, (LANES, LANES), 1) // HD
            for j in range(NG):
                gs = slice((j // 2) * LANES, (j // 2 + 1) * LANES)
                gl, gr = (g11, g12) if j % 2 == 0 else (g21, g22)
                gj = jnp.concatenate([gl[gs], gr[gs]], axis=1).astype(BF16)
                kv = _dot(gj, wv_v[:, j * LANES:(j + 1) * LANES])
                kvs.append(jnp.where(r == c, kv, 0.0).astype(BF16))

        def state_m():
            perm_store(jnp.concatenate([_dot(kvs[j], wo_v[j * LANES:(j + 1) * LANES, :]) for j in range(NG)],
                                       axis=0), 2 * NG)
            del jobs[-(H // STRIP):]
            for n, k0 in enumerate(range(0, H, STRIP)):
                jobs.insert(10 + 3 * n, one_level_job(lambda r, c, k0=k0: jnp.concatenate(
                    [perm_load((2 + r) * NG + 2 * c + l, k0, STRIP) for l in range(2)], axis=1), d1_v, LANES + k0))

        def odd_chunk(t, hooks):
            m = [None] * 7
            for k, i in enumerate(ORDER):
                if k in hooks:
                    hooks[k]()
                m[i] = _dot(x_op(i, t * TS, TS), load2(g1_v, i, 0, H))
                run_jobs(m[i], H)
            for q, c in enumerate(_out4(m)):
                h1_v[q // 2, t * TS:(t + 1) * TS, (q % 2) * LANES:(q % 2 + 1) * LANES] = _silu_mul(c, 0.5)

        def prologue():
            wait_group(0)
            wk_prep(0)
            wait_group(1)
            for p0 in range(0, STAGES[0], LANES):
                kg(p0, 0, 1, p0 == 0, True)
            wait_group(2)
            wk_prep(1)
            for p0 in range(STAGES[0], STAGES[1], LANES):
                kg(p0, 0, 1, False, True)
            for p0 in range(0, STAGES[1], LANES):
                kg(p0, 1, 2, p0 == 0, False)
            wait_group(3)
            for p0 in range(STAGES[1], STAGES[2], LANES):
                kg(p0, 0, 2, False, True)

            wait_group(4)
            n1, n2 = permuted(wq_v[...].T.astype(F32), 0)
            sq = [u.astype(BF16) for u in _rhs7(n1[:, :H], n2[:, :H], n1[:, H:], n2[:, H:])]
            gate_up_weight_jobs()
            plan(14 * (P - STAGES[2]) + 7 * P, 14 * (P - STAGES[2]), 300)
            for p0 in range(STAGES[2], P, LANES):
                kg(p0, 0, 2, False, True)
            rows_prep()
            for i in ORDER_Q:
                m = _dot_nt(x_op(i, 0, P), sq[i])
                run_jobs(m, H)
                q_v[i] = m
            assert not jobs

            wait_group(SEM_W)
            gate_jobs(0)
            x_tile_jobs(0)
            down_weight_jobs()
            jobs.extend([None] * (H // STRIP))
            plan(7 * P, 0, 150)
            for t in range(NT):
                odd_chunk(t, {3: state_kv, 6: state_m} if t == 0 else {})
            assert not jobs

        def gate_up(row, zero):
            light_outer, light_inner = (0, 2, 4), (0, 1, 2, 3, 4, 5)
            attn_jobs(row, zero)
            plan(NPAIR * len(light_outer) * len(light_inner) * HN // 2, 0, 1)
            for p in range(NPAIR):
                mo = [None] * 7
                for ko, i in enumerate(ORDER):
                    m = [None] * 7
                    for ki, j in enumerate(ORDER):
                        m[j] = _dot(t2_v[7 * i + j], load2(g2_v, 49 * p + 7 * i + j, 0, LANES))
                        if ko in light_outer and ki in light_inner:
                            run_jobs(m[j], LANES)
                    mo[i] = _out4(m)
                c16 = [_out4([mo[i][inner] for i in range(7)]) for inner in range(4)]
                for q in QUADS:
                    for inner in QUADS:
                        r, c = divmod(inner, 2)
                        c0 = (q % 2) * FL + p * H + c * LANES
                        h_v[q // 2, at(row, r * HN, HN), c0:c0 + LANES] = _silu_mul(
                            c16[inner][q], cg_v[q // 2, r * HN:(r + 1) * HN, :])
            assert not jobs

        def emit(hf, rows, c0, cn):
            pltpu.make_async_copy(out_v.at[hf, rows, pl.ds(c0, cn)], out_hbm.at[hf, rows, pl.ds(c0, cn)],
                                  sem.at[SEM_O]).start()

        def down(row, nxt):
            K1 = LANES + H
            AHEAD, WEIGHT = 3, 4.0

            def hblk(R, C, r, c):
                return jnp.concatenate(
                    [h_v[R, at(row, r * HN, HN), C * FL + p * H + c * LANES:C * FL + p * H + (c + 1) * LANES]
                     for p in range(NPAIR)], axis=1)
            v = [u.astype(BF16) for u in _lhs7(*[pn_v[R, :, C * K1:(C + 1) * K1] for R in range(2) for C in range(2)])]
            x_tile_jobs(nxt)
            gate_jobs(nxt)
            plan(49 * NPAIR * HN // 4 + WEIGHT * 7 * 6 * TS // 4, 300, 400)
            m1 = [None] * 7

            def one_level(k):
                if k < 7:
                    m1[ORDER[k]] = _dot(v[ORDER[k]], load2(d1_v, ORDER[k], 0, K1))
                    run_jobs(m1[ORDER[k]], K1, WEIGHT)
            for k in range(AHEAD - 1):
                one_level(k)
            mo = [None] * 7
            done = set()
            for ko, i in enumerate(ORDER):
                one_level(AHEAD - 1 + ko)
                a = _lhs7(*[_combine(L_TERMS[i], lambda R, C: hblk(R, C, r, c)) for r in range(2) for c in range(2)])
                m = [None] * 7
                for j in ORDER:
                    m[j] = _dot(a[j].astype(BF16), d2_v[7 * i + j])
                    run_jobs(m[j], NPAIR * LANES)
                mo[i] = [c + m1[i][(k // 2) * HN:(k // 2 + 1) * HN, (k % 2) * LANES:(k % 2 + 1) * LANES]
                         for k, c in enumerate(_out4(m))]
                for q in QUADS:
                    if q in done or any(mo[t[0]] is None for t in C_TERMS[q]):
                        continue
                    done.add(q)
                    o = [_combine(C_TERMS[q], lambda kk: mo[kk][k]) for k in range(4)]
                    c0 = (q % 2) * H
                    if q == QUADS[-1]:
                        for k in QUADS:
                            rows, c1 = at(row, (k // 2) * HN, HN), c0 + (k % 2) * LANES
                            out_v[q // 2, rows, c1:c1 + LANES] = o[k].astype(BF16)
                            emit(q // 2, rows, c1, LANES)
                    else:
                        for r in range(2):
                            out_v[q // 2, at(row, r * HN, HN), c0:c0 + H] = jnp.concatenate(
                                o[2 * r:2 * r + 2], axis=1).astype(BF16)
                        emit(q // 2, at(row, 0, TS), c0, H)
            assert not jobs

        def tile(i, carry):
            pl.when(i == 0)(prologue)
            row = pl.multiple_of(i * TS, TS)
            gate_up(row, i // NT)
            down(row, pl.multiple_of(jnp.minimum(i + 1, NT - 1) * TS, TS))
            return carry

        lax.fori_loop(0, NT, tile, 0)
        pltpu.make_async_copy(out_v, out_hbm, sem.at[SEM_O]).wait()

    any_spec = pl.BlockSpec(memory_space=pl.ANY)
    out = pl.pallas_call(
        kernel,
        out_shape=jax.ShapeDtypeStruct((2, P, D), BF16),
        in_specs=[any_spec] * 7,
        out_specs=any_spec,
        scratch_shapes=[
            pltpu.VMEM((2, P, D), BF16),
            pltpu.VMEM((D, D), BF16),
            pltpu.VMEM((D, D), BF16),
            pltpu.VMEM((D, D), BF16),
            pltpu.VMEM((D, D), BF16),
            pltpu.VMEM((D, F), BF16),
            pltpu.VMEM((D, F), BF16),
            pltpu.VMEM((F, D), BF16),
            pltpu.VMEM((D,), BF16),
            pltpu.VMEM((14, P, LANES), BF16),
            pltpu.VMEM((49, HN, LANES), BF16),
            pltpu.VMEM((14, H, LANES), BF16),
            pltpu.VMEM((14, H, LANES), BF16),
            pltpu.VMEM((14, LANES + H, LANES), BF16),
            pltpu.VMEM((NPAIR * 49 * 2, LANES, LANES), BF16),
            pltpu.VMEM((49, NPAIR * LANES, LANES), BF16),
            pltpu.VMEM((7, H, H), F32),
            pltpu.VMEM((D, LANES), F32),
            pltpu.VMEM((4 * NG + 2, H + 32, LANES), F32),
            pltpu.VMEM((7, P, H), F32),
            pltpu.VMEM((16, D), F32),
            pltpu.VMEM((2, P, 2 * LANES), F32),
            pltpu.VMEM((2, P, 2 * FL), F32),
            pltpu.VMEM((2, TS, 2 * (LANES + H)), F32),
            pltpu.VMEM((2, TS, LANES), F32),
            pltpu.VMEM((2, P, D), BF16),
            pltpu.SemaphoreType.DMA((NS + 3,)),
        ],
        compiler_params=pltpu.CompilerParams(
            vmem_limit_bytes=110 * 1024 * 1024,
            **{k: True for k in ("disable_bounds_checks", "disable_semaphore_checks")
               if hasattr(pltpu.CompilerParams, k)},
        ),
    )(A_x.reshape(2, P, D), A_wqkv, A_wo, B_w_gate, B_w_up, B_w_down, gate_w)
    return out.reshape(B, S, D)
```
